```python
import os as _os
_os.environ.setdefault("JAX_PLATFORMS", "cpu")
import jax
import jax.numpy as jnp

def _softmax(x, axis=-1):
    return jax.nn.softmax(x, axis=axis)
def _gelu(x):
    return jax.nn.gelu(x, approximate=True)
def _silu(x):
    return jax.nn.silu(x)
def _sigmoid(x):
    return jax.nn.sigmoid(x)
def _layernorm(x, axis=-1, eps=1e-5):
    m = jnp.mean(x, axis=axis, keepdims=True)
    v = jnp.var(x, axis=axis, keepdims=True)
    return (x - m) / jnp.sqrt(v + eps)
def _scatter_add(tgt, idx, src, axis=0):
    return tgt.at[idx].add(src)
def _segment_sum(src, seg, n):
    return jax.ops.segment_sum(src, seg, n)
class _Rng:
    def __init__(self, key):
        self._k = key
    def _next(self):
        self._k, sub = jax.random.split(self._k)
        return sub
    def normal(self, shape):
        return jax.random.normal(self._next(), shape, dtype=jnp.bfloat16)
    def randint(self, lo, hi, shape):
        return jax.random.randint(self._next(), shape, lo, hi, dtype=jnp.int32)
    def uniform(self, shape, lo=0.0, hi=1.0):
        return jax.random.uniform(self._next(), shape, jnp.bfloat16, lo, hi)
    def permutation(self, n):
        return jax.random.permutation(self._next(), n)


kernel_name = 'concat_heads__mha_block_cached__mha_block_cached__near_ridge'

def setup_inputs():
    _rng = _Rng(jax.random.key(int.from_bytes(__import__("os").urandom(4), "little")))
    _w = (lambda a: (lambda t: t.astype(jnp.bfloat16) if jnp.issubdtype(t.dtype, jnp.floating) else t)(jnp.asarray(a)))
    def _A_setup():
        B, Sq, D = 16, 80, 512
        H, Sk, Dh = 32, 80, 128
        return {
            "x": _w((lambda *s: _rng.normal(s) * 0.8)(B, Sq, D)),
            "k_cache": _w((lambda *s: _rng.normal(s) * 0.8)(B, H, Sk, Dh)),
            "v_cache": _w((lambda *s: _rng.normal(s) * 0.05)(B, H, Sk, Dh)),
            "wq": _w((lambda *s: _rng.normal(s) * 0.8)(D, H * Dh) * (D ** -0.5)),
            "wo": _w((lambda *s: _rng.normal(s) * 0.05)(H * Dh, D) * ((H * Dh) ** -0.5)),
        }
    _A_in = _A_setup()

    def _B_setup():
        B, Sq, D = 16, 80, 512
        H, Sk, Dh = 32, 80, 128
        return {
            "x": _w((lambda *s: _rng.normal(s) * 0.8)(B, Sq, D)),
            "k_cache": _w((lambda *s: _rng.normal(s) * 0.8)(B, H, Sk, Dh)),
            "v_cache": _w((lambda *s: _rng.normal(s) * 0.05)(B, H, Sk, Dh)),
            "wq": _w((lambda *s: _rng.normal(s) * 0.8)(D, H * Dh) * (D ** -0.5)),
            "wo": _w((lambda *s: _rng.normal(s) * 0.05)(H * Dh, D) * ((H * Dh) ** -0.5)),
        }
    _B_in = _B_setup()

    return {
        "A_x": _A_in["x"],
        "A_k_cache": _A_in["k_cache"],
        "A_v_cache": _A_in["v_cache"],
        "A_wq": _A_in["wq"],
        "A_wo": _A_in["wo"],
        "B_x": _B_in["x"],
        "B_k_cache": _B_in["k_cache"],
        "B_v_cache": _B_in["v_cache"],
        "B_wq": _B_in["wq"],
        "B_wo": _B_in["wo"],
    }

def reference(A_x, A_k_cache, A_v_cache, A_wq, A_wo, B_x, B_k_cache, B_v_cache, B_wq, B_wo):
    def _A_ref(x, k_cache, v_cache, wq, wo):
        B, Sq, D = x.shape
        H, Dh = 32, 128
        q = (lambda x, *d: x.transpose(*d))((x @ wq).reshape(B, Sq, H, Dh), 0, 2, 1, 3)
        scores = jnp.einsum("bhqd,bhkd->bhqk", q, k_cache) * (Dh ** -0.5)
        p = _softmax(scores, axis=-1)
        o = jnp.einsum("bhqk,bhkd->bhqd", p, v_cache)
        return (lambda x, *d: x.transpose(*d))(o, 0, 2, 1, 3).reshape(B, Sq, H * Dh) @ wo

    def _B_ref(x, k_cache, v_cache, wq, wo):
        B, Sq, D = x.shape
        H, Dh = 32, 128
        q = (lambda x, *d: x.transpose(*d))((x @ wq).reshape(B, Sq, H, Dh), 0, 2, 1, 3)
        scores = jnp.einsum("bhqd,bhkd->bhqk", q, k_cache) * (Dh ** -0.5)
        p = _softmax(scores, axis=-1)
        o = jnp.einsum("bhqk,bhkd->bhqd", p, v_cache)
        return (lambda x, *d: x.transpose(*d))(o, 0, 2, 1, 3).reshape(B, Sq, H * Dh) @ wo

    a = _A_ref(A_x, A_k_cache, A_v_cache, A_wq, A_wo)
    b = _B_ref(B_x, B_k_cache, B_v_cache, B_wq, B_wo)
    return jnp.concatenate([a, b], axis=-1)
```

```python
import functools
import contextlib
import jax
import jax.numpy as jnp
import jax.experimental.pallas as pl
import jax.experimental.pallas.tpu as pltpu

B, SQ, D = 16, 80, 512
H, SK, DH = 32, 80, 128
M = B * SQ
LOG2E = 1.4426950408889634
NC = 4
BPC = B // NC
RC = BPC * SQ
F32 = jnp.float32
BF16 = jnp.bfloat16


def impl(A_x, A_k, A_v, A_wq, A_wo, B_x, B_k, B_v, B_wq, B_wo, HPB=4, ORDER="kqpo", LORDER="kop", OR=2,
         SC=False, STARTPOS=1, TAILSPLIT=4):
    TPB = H // HPB
    NT = 2 * TPB
    UPB = HPB * NC
    cexp = (DH ** -0.5) * LOG2E
    assert UPB % OR == 0
    scope = jax.named_scope if SC else (lambda n: contextlib.nullcontext())

    def kernel(ax, ak, av, awq, awo, bx, bk, bv, bwq, bwo, out_hbm,
               x_all, k_all, v_all, wq_all, wo_all, q_buf, o_ring, acc, stage,
               sem_x, sem_k, sem_v, sem_wq, sem_wo, sem_h, sem_out):

        def srcs(br):
            return (ak, av, awq, awo) if br == 0 else (bk, bv, bwq, bwo)

        def col0(h):
            return h * DH if isinstance(h, int) else pl.multiple_of(h * DH, DH)

        def grp_copy(name, T, br):
            kk, vv, wq, wo = srcs(br)
            h0 = (T - br * TPB) * HPB
            if name == "k":
                return pltpu.make_async_copy(kk.at[:, pl.ds(h0, HPB)], k_all.at[T], sem_k.at[T])
            if name == "v":
                return pltpu.make_async_copy(vv.at[:, pl.ds(h0, HPB)], v_all.at[T], sem_v.at[T])
            if name == "wq":
                return pltpu.make_async_copy(wq.at[:, pl.ds(col0(h0), HPB * DH)], wq_all.at[T], sem_wq.at[T])
            return pltpu.make_async_copy(wo.at[pl.ds(col0(h0), HPB * DH), :], wo_all.at[T], sem_wo.at[T])

        def start_grp(names, T):
            if isinstance(T, int):
                if T < NT:
                    for n in names:
                        grp_copy(n, T, 0 if T < TPB else 1).start()
            else:
                @pl.when(T < TPB)
                def _():
                    for n in names:
                        grp_copy(n, T, 0).start()

                @pl.when(jnp.logical_and(T >= TPB, T < NT))
                def _():
                    for n in names:
                        grp_copy(n, T, 1).start()

        def wait_grp(ref_all, sem, T):
            pltpu.make_async_copy(ref_all.at[T], ref_all.at[T], sem.at[T]).wait()

        def head_copy(name, j):
            if name == "wq0":
                return pltpu.make_async_copy(awq.at[:, pl.ds(col0(j), DH)], wq_all.at[0, :, pl.ds(col0(j), DH)], sem_h.at[j])
            if name == "wq1":
                return pltpu.make_async_copy(awq.at[:, pl.ds(col0(HPB + j), DH)], wq_all.at[1, :, pl.ds(col0(j), DH)], sem_h.at[HPB + j])
            if name == "k":
                return pltpu.make_async_copy(ak.at[:, j], k_all.at[0, :, j], sem_h.at[2 * HPB + j])
            if name == "v":
                return pltpu.make_async_copy(av.at[:, j], v_all.at[0, :, j], sem_h.at[3 * HPB + j])
            return pltpu.make_async_copy(awo.at[pl.ds(col0(j), DH), :], wo_all.at[0, pl.ds(col0(j), DH), :], sem_h.at[4 * HPB + j])

        def x_copy(br, c):
            src = ax if br == 0 else bx
            r0 = c * RC if isinstance(c, int) else pl.multiple_of(c * RC, RC)
            return pltpu.make_async_copy(src.at[pl.ds(r0, RC)], x_all.at[br, pl.ds(r0, RC)], sem_x.at[br * NC + c])

        def out_copy(br, r0, nr, s):
            return pltpu.make_async_copy(stage.at[br, pl.ds(r0, nr)], out_hbm.at[pl.ds(r0, nr), pl.ds(br * D, D)], sem_out.at[s])

        def qproj(u, T):
            j, c = divmod(u, NC)
            br = T // TPB
            xs = x_all[br, pl.ds(c * RC, RC), :]
            q = jnp.dot(xs, wq_all[T, :, pl.ds(j * DH, DH)], preferred_element_type=F32)
            q_buf[u] = q.astype(BF16)

        def qk_softmax(u, T):
            j, c = divmod(u, NC)
            ps = []
            for i in range(BPC):
                q = q_buf[u, pl.ds(i * SQ, SQ), :]
                k = k_all[T, c * BPC + i, j]
                s = jax.lax.dot_general(q, k, (((1,), (1,)), ((), ())), preferred_element_type=F32)
                m = jnp.max(s, axis=-1, keepdims=True)
                p = jnp.exp2((s - m) * cexp)
                l = jnp.sum(p, axis=-1, keepdims=True)
                ps.append((p.astype(BF16), pl.reciprocal(l, approx=True)))
            return ps

        def pv(ps, u, T):
            j, c = divmod(u, NC)
            for i in range(BPC):
                p, r = ps[i]
                o = jnp.dot(p, v_all[T, c * BPC + i, j], preferred_element_type=F32)
                o_ring[u % OR, pl.ds(i * SQ, SQ), :] = (o * r).astype(BF16)

        def oproj(u, T, mode="acc", r0=0, nr=RC):
            To = T - 1 if u < 0 else T
            j, c = divmod(u % UPB, NC)
            br = To // TPB
            part = jnp.dot(o_ring[u % OR, pl.ds(r0, nr), :], wo_all[To, pl.ds(j * DH, DH), :], preferred_element_type=F32)
            rows = pl.ds(c * RC + r0, nr)
            if mode == "acc":
                acc[br, rows, :] += part
            elif mode == "first":
                acc[br, rows, :] = part
            else:
                stage[br, rows, :] = (acc[br, rows, :] + part).astype(BF16)

        with scope("pro_start"):
            x_copy(0, 0).start()
            head_copy("wq0", 0).start()

            def s_wq0(j, _):
                head_copy("wq0", j).start()
                return 0
            jax.lax.fori_loop(1, HPB, s_wq0, 0)

            def s_x(c, _):
                x_copy(0, c).start()
                return 0
            jax.lax.fori_loop(1, NC, s_x, 0)

            def s_head(j, _):
                head_copy("k", j).start()
                head_copy("v", j).start()
                head_copy("wq1", j).start()
                head_copy("wo", j).start()
                return 0
            jax.lax.fori_loop(0, HPB, s_head, 0)
            start_grp(["k", "v", "wo"], 1)
            start_grp(["wq"], 2)
        with scope("pro_zero"):
            acc[1] = jnp.zeros(acc.shape[1:], F32)
        with scope("pro_q"):
            for c in range(NC):
                x_copy(0, c).wait()
                for j in range(HPB):
                    if c == 0:
                        head_copy("wq0", j).wait()
                    qproj(j * NC + c, 0)

        def units(T, kind):
            order = LORDER if kind == "last" else ORDER
            for u in range(UPB):
                j, c = divmod(u, NC)
                if kind == "first" and c == 0:
                    for n in ("k", "v", "wq1", "wo"):
                        head_copy(n, j).wait()
                if u == STARTPOS and kind != "last":
                    start_grp(["k", "v", "wo"], T + 2)
                    start_grp(["wq"], T + 3)
                    if kind == "first":
                        for cc in range(NC):
                            x_copy(1, cc).start()
                ps = None
                for op in order:
                    if op == "k":
                        ps = qk_softmax(u, T)
                    elif op == "q":
                        qproj(u, T + 1)
                    elif op == "p":
                        pv(ps, u, T)
                    elif op == "o":
                        if kind == "first":
                            if u >= 1:
                                oproj(u - 1, T, "first" if u - 1 < NC else "acc")
                        elif kind == "last" and u - 1 >= UPB - NC:
                            oproj(u - 1, T, "final")
                            cc = (u - 1) % NC
                            out_copy(1, cc * RC, RC, 1 + cc).start()
                        else:
                            oproj(u - 1, T)

        with scope("first"):
            units(0, "first")

        def body(T, carry):
            with scope("waits"):
                wait_grp(k_all, sem_k, T)
                wait_grp(v_all, sem_v, T)
                wait_grp(wo_all, sem_wo, T)
                wait_grp(wq_all, sem_wq, T + 1)

                @pl.when(T == TPB - 1)
                def _():
                    for c in range(NC):
                        x_copy(1, c).wait()

            with scope("units"):
                units(T, "mid")

            with scope("finA"):
                @pl.when(T == TPB)
                def _():
                    stage[0] = acc[0].astype(BF16)
                    out_copy(0, 0, M, 0).start()
            return carry

        with scope("mainloop"):
            jax.lax.fori_loop(1, NT - 1, body, 0)
        with scope("last"):
            T = NT - 1
            wait_grp(k_all, sem_k, T)
            wait_grp(v_all, sem_v, T)
            wait_grp(wo_all, sem_wo, T)
            units(T, "last")
        with scope("epilogue"):
            nr = RC // TAILSPLIT
            for s in range(TAILSPLIT):
                oproj(UPB - 1, NT - 1, "final", r0=s * nr, nr=nr)
                out_copy(1, (NC - 1) * RC + s * nr, nr, NC + s).start()
            out_copy(0, 0, M, 0).wait()
            for cc in range(NC - 1):
                out_copy(1, cc * RC, RC, 1 + cc).wait()
            for s in range(TAILSPLIT):
                out_copy(1, (NC - 1) * RC + s * nr, nr, NC + s).wait()

    any_spec = pl.BlockSpec(memory_space=pl.ANY)
    out = pl.pallas_call(
        kernel,
        in_specs=[any_spec] * 10,
        out_specs=any_spec,
        out_shape=jax.ShapeDtypeStruct((M, 2 * D), BF16),
        scratch_shapes=[
            pltpu.VMEM((2, M, D), BF16),
            pltpu.VMEM((NT, B, HPB, SK, DH), BF16),
            pltpu.VMEM((NT, B, HPB, SK, DH), BF16),
            pltpu.VMEM((NT, D, HPB * DH), BF16),
            pltpu.VMEM((NT, HPB * DH, D), BF16),
            pltpu.VMEM((UPB, RC, DH), BF16),
            pltpu.VMEM((OR, RC, DH), BF16),
            pltpu.VMEM((2, M, D), F32),
            pltpu.VMEM((2, M, D), BF16),
            pltpu.SemaphoreType.DMA((2 * NC,)),
            pltpu.SemaphoreType.DMA((NT,)),
            pltpu.SemaphoreType.DMA((NT,)),
            pltpu.SemaphoreType.DMA((NT,)),
            pltpu.SemaphoreType.DMA((NT,)),
            pltpu.SemaphoreType.DMA((5 * HPB,)),
            pltpu.SemaphoreType.DMA((NC + TAILSPLIT,)),
        ],
        compiler_params=pltpu.CompilerParams(vmem_limit_bytes=110 * 1024 * 1024, disable_bounds_checks=True),
    )(A_x.reshape(M, D), A_k, A_v, A_wq, A_wo, B_x.reshape(M, D), B_k, B_v, B_wq, B_wo)
    return out.reshape(B, SQ, 2 * D)


@jax.jit
def pallas_concat_heads__mha_block_cached__mha_block_cached__near_ridge_kernel(
        A_x, A_k_cache, A_v_cache, A_wq, A_wo, B_x, B_k_cache, B_v_cache, B_wq, B_wo):
    return impl(A_x, A_k_cache, A_v_cache, A_wq, A_wo, B_x, B_k_cache, B_v_cache, B_wq, B_wo)
```

```python
import contextlib
import jax
import jax.numpy as jnp
import jax.experimental.pallas as pl
import jax.experimental.pallas.tpu as pltpu

B, SQ, D = 16, 80, 512
H, SK, DH = 32, 80, 128
M = B * SQ
LOG2E = 1.4426950408889634
NC = 4
BPC = B // NC
RC = BPC * SQ
F32 = jnp.float32
BF16 = jnp.bfloat16


def impl(A_x, A_k, A_v, A_wq, A_wo, B_x, B_k, B_v, B_wq, B_wo, HPB=4, ORDER="kqpo", OR=4,
         SC=False, STARTPOS=1, TAILSPLIT=4, RCP="newton", CMAJ=True, FOLD=True, PRO=2):
    TPB = H // HPB
    NT = 2 * TPB
    UPB = HPB * NC
    cexp = (DH ** -0.5) * LOG2E
    assert UPB % OR == 0
    scope = jax.named_scope if SC else (lambda n: contextlib.nullcontext())

    def kernel(ax, ak, av, awq, awo, bx, bk, bv, bwq, bwo, out_hbm,
               x_all, k_all, v_all, wq_all, wo_all, q_buf, o_ring, acc, stage,
               sem_x, sem_k, sem_v, sem_wq, sem_wo, sem_h, sem_out):

        def srcs(br):
            return (ak, av, awq, awo) if br == 0 else (bk, bv, bwq, bwo)

        def col0(h):
            return h * DH if isinstance(h, int) else pl.multiple_of(h * DH, DH)

        def grp_copy(name, T, br):
            kk, vv, wq, wo = srcs(br)
            h0 = (T - br * TPB) * HPB
            if name == "k":
                return pltpu.make_async_copy(kk.at[:, pl.ds(h0, HPB)], k_all.at[T], sem_k.at[T])
            if name == "v":
                return pltpu.make_async_copy(vv.at[:, pl.ds(h0, HPB)], v_all.at[T], sem_v.at[T])
            if name == "wq":
                return pltpu.make_async_copy(wq.at[:, pl.ds(col0(h0), HPB * DH)], wq_all.at[T], sem_wq.at[T])
            return pltpu.make_async_copy(wo.at[pl.ds(col0(h0), HPB * DH), :], wo_all.at[T], sem_wo.at[T])

        def start_grp(names, T):
            if isinstance(T, int):
                if T < NT:
                    for n in names:
                        grp_copy(n, T, 0 if T < TPB else 1).start()
            else:
                @pl.when(T < TPB)
                def _():
                    for n in names:
                        grp_copy(n, T, 0).start()

                @pl.when(jnp.logical_and(T >= TPB, T < NT))
                def _():
                    for n in names:
                        grp_copy(n, T, 1).start()

        def wait_grp(ref_all, sem, T):
            pltpu.make_async_copy(ref_all.at[T], ref_all.at[T], sem.at[T]).wait()

        def head_copy(name, j):
            if name == "wq0":
                return pltpu.make_async_copy(awq.at[:, pl.ds(col0(j), DH)], wq_all.at[0, :, pl.ds(col0(j), DH)], sem_h.at[j])
            if name == "wq1":
                return pltpu.make_async_copy(awq.at[:, pl.ds(col0(HPB + j), DH)], wq_all.at[1, :, pl.ds(col0(j), DH)], sem_h.at[HPB + j])
            if name == "k":
                return pltpu.make_async_copy(ak.at[:, j], k_all.at[0, :, j], sem_h.at[2 * HPB + j])
            if name == "v":
                return pltpu.make_async_copy(av.at[:, j], v_all.at[0, :, j], sem_h.at[3 * HPB + j])
            return pltpu.make_async_copy(awo.at[pl.ds(col0(j), DH), :], wo_all.at[0, pl.ds(col0(j), DH), :], sem_h.at[4 * HPB + j])

        def x_copy(br, c):
            src = ax if br == 0 else bx
            r0 = c * RC if isinstance(c, int) else pl.multiple_of(c * RC, RC)
            return pltpu.make_async_copy(src.at[pl.ds(r0, RC)], x_all.at[br, pl.ds(r0, RC)], sem_x.at[br * NC + c])

        def out_copy(br, r0, nr, s):
            return pltpu.make_async_copy(stage.at[br, pl.ds(r0, nr)], out_hbm.at[pl.ds(r0, nr), pl.ds(br * D, D)], sem_out.at[s])

        def qproj(u, T):
            j, c = divmod(u, NC)
            br = T // TPB
            xs = x_all[br, pl.ds(c * RC, RC), :]
            q = jnp.dot(xs, wq_all[T, :, pl.ds(j * DH, DH)], preferred_element_type=F32)
            q_buf[u] = q.astype(BF16)

        def qk_softmax(u, T):
            j, c = divmod(u, NC)
            ps = []
            for i in range(BPC):
                q = q_buf[u, pl.ds(i * SQ, SQ), :]
                k = k_all[T, c * BPC + i, j]
                s = jax.lax.dot_general(q, k, (((1,), (1,)), ((), ())), preferred_element_type=F32)
                m = jnp.max(s, axis=-1, keepdims=True)
                p = jnp.exp2((s - m) * cexp)
                l = jnp.sum(p, axis=-1, keepdims=True)
                r = pl.reciprocal(l, approx=True)
                if RCP == "newton":
                    r = r * (2.0 - l * r)
                ps.append((p.astype(BF16), r))
            return ps

        def pv(ps, u, T, slot=None):
            slot = u % OR if slot is None else slot
            j, c = divmod(u, NC)
            for i in range(BPC):
                p, r = ps[i]
                o = jnp.dot(p, v_all[T, c * BPC + i, j], preferred_element_type=F32)
                o_ring[slot, pl.ds(i * SQ, SQ), :] = (o * r).astype(BF16)

        def oproj(u, T, mode="acc", r0=0, nr=RC, slot=None):
            slot = u % OR if slot is None else slot
            To = T - 1 if u < 0 else T
            j, c = divmod(u % UPB, NC)
            br = To // TPB
            part = jnp.dot(o_ring[slot, pl.ds(r0, nr), :], wo_all[To, pl.ds(j * DH, DH), :], preferred_element_type=F32)
            rows = pl.ds(c * RC + r0, nr)
            if mode == "first":
                acc[br, rows, :] = part
            elif mode == "final":
                stage[br, rows, :] = (acc[br, rows, :] + part).astype(BF16)
            else:
                new = acc[br, rows, :] + part
                acc[br, rows, :] = new
                if FOLD and j == HPB - 1:
                    stage[br, rows, :] = new.astype(BF16)

        def wait_heads(js):
            for j in js:
                for n in ("k", "v", "wq1", "wo"):
                    head_copy(n, j).wait()

        with scope("pro_start"):
            x_copy(0, 0).start()
            head_copy("wq0", 0).start()

            def s_wq0(j, _):
                head_copy("wq0", j).start()
                return 0
            jax.lax.fori_loop(1, HPB, s_wq0, 0)

            def s_x(c, _):
                x_copy(0, c).start()
                return 0
            jax.lax.fori_loop(1, NC, s_x, 0)

            def s_head(j, _):
                head_copy("k", j).start()
                head_copy("v", j).start()
                head_copy("wq1", j).start()
                head_copy("wo", j).start()
                return 0
            jax.lax.fori_loop(0, HPB, s_head, 0)
            start_grp(["k", "v", "wo"], 1)
            start_grp(["wq"], 2)
        with scope("pro_zero"):
            acc[1] = jnp.zeros(acc.shape[1:], F32)
        with scope("pro_q"):
            if PRO == 1:
                for c in range(NC):
                    x_copy(0, c).wait()
                    for j in range(HPB):
                        if c == 0:
                            head_copy("wq0", j).wait()
                        qproj(j * NC + c, 0)
            else:
                hh = HPB // 2
                x_copy(0, 0).wait()
                for j in range(hh):
                    head_copy("wq0", j).wait()
                for j in range(hh):
                    qproj(j * NC, 0)
                for j in range(hh, HPB):
                    head_copy("wq0", j).wait()
                x_copy(0, 1).wait()
                for j in range(hh, HPB):
                    qproj(j * NC, 0)
                for j in range(HPB):
                    qproj(j * NC + 1, 0)
                x_copy(0, 2).wait()
                x_copy(0, 3).wait()
                for c in range(2, NC):
                    for j in range(HPB):
                        qproj(j * NC + c, 0)

        def units(T, kind):
            for u in range(UPB):
                j, c = divmod(u, NC)
                if kind == "first" and c == 0:
                    if PRO == 1:
                        wait_heads([j])
                    elif j % 2 == 0:
                        wait_heads([j, j + 1])
                if u == STARTPOS:
                    start_grp(["k", "v", "wo"], T + 2)
                    start_grp(["wq"], T + 3)
                    if kind == "first":
                        for cc in range(NC):
                            x_copy(1, cc).start()
                    elif FOLD:
                        @pl.when(T == TPB)
                        def _():
                            out_copy(0, 0, M, 0).start()
                ps = None
                for op in ORDER:
                    if op == "k":
                        ps = qk_softmax(u, T)
                    elif op == "q":
                        qproj(u, T + 1)
                    elif op == "p":
                        pv(ps, u, T)
                    elif op == "o":
                        if kind == "first":
                            if u >= 1:
                                oproj(u - 1, T, "first" if u - 1 < NC else "acc")
                        else:
                            oproj(u - 1, T)

        def last_units(T):
            order = [j * NC + c for c in range(NC) for j in range(HPB)] if CMAJ else list(range(UPB))
            slot = {u: i % OR for i, u in enumerate(order)}
            slot[-1] = (UPB - 1) % OR

            def o_last(u):
                if u >= UPB - NC:
                    cc = u % NC
                    if u == UPB - 1:
                        nr = RC // TAILSPLIT
                        for s in range(TAILSPLIT):
                            oproj(u, T, "final", r0=s * nr, nr=nr, slot=slot[u])
                            out_copy(1, cc * RC + s * nr, nr, NC + s).start()
                    else:
                        oproj(u, T, "final", slot=slot[u])
                        out_copy(1, cc * RC, RC, 1 + cc).start()
                else:
                    oproj(u, T, slot=slot[u])
            pss = {}
            pss[0] = qk_softmax(order[0], T)
            pss[1] = qk_softmax(order[1], T)
            o_last(-1)
            pv(pss.pop(0), order[0], T, slot=slot[order[0]])
            for s in range(2, UPB):
                pss[s] = qk_softmax(order[s], T)
                pv(pss.pop(s - 1), order[s - 1], T, slot=slot[order[s - 1]])
                o_last(order[s - 2])
            pv(pss.pop(UPB - 1), order[UPB - 1], T, slot=slot[order[UPB - 1]])
            o_last(order[UPB - 2])
            o_last(order[UPB - 1])

        with scope("first"):
            units(0, "first")

        def body(T, carry):
            with scope("waits"):
                wait_grp(k_all, sem_k, T)
                wait_grp(v_all, sem_v, T)
                wait_grp(wo_all, sem_wo, T)
                wait_grp(wq_all, sem_wq, T + 1)

                @pl.when(T == TPB - 1)
                def _():
                    for c in range(NC):
                        x_copy(1, c).wait()

            with scope("units"):
                units(T, "mid")

            if not FOLD:
                with scope("finA"):
                    @pl.when(T == TPB)
                    def _():
                        stage[0] = acc[0].astype(BF16)
                        out_copy(0, 0, M, 0).start()
            return carry

        with scope("mainloop"):
            jax.lax.fori_loop(1, NT - 1, body, 0)
        with scope("last"):
            T = NT - 1
            wait_grp(k_all, sem_k, T)
            wait_grp(v_all, sem_v, T)
            wait_grp(wo_all, sem_wo, T)
            last_units(T)
        with scope("epilogue"):
            nr = RC // TAILSPLIT
            out_copy(0, 0, M, 0).wait()
            for cc in range(NC - 1):
                out_copy(1, cc * RC, RC, 1 + cc).wait()
            for s in range(TAILSPLIT):
                out_copy(1, (NC - 1) * RC + s * nr, nr, NC + s).wait()

    any_spec = pl.BlockSpec(memory_space=pl.ANY)
    out = pl.pallas_call(
        kernel,
        in_specs=[any_spec] * 10,
        out_specs=any_spec,
        out_shape=jax.ShapeDtypeStruct((M, 2 * D), BF16),
        scratch_shapes=[
            pltpu.VMEM((2, M, D), BF16),
            pltpu.VMEM((NT, B, HPB, SK, DH), BF16),
            pltpu.VMEM((NT, B, HPB, SK, DH), BF16),
            pltpu.VMEM((NT, D, HPB * DH), BF16),
            pltpu.VMEM((NT, HPB * DH, D), BF16),
            pltpu.VMEM((UPB, RC, DH), BF16),
            pltpu.VMEM((OR, RC, DH), BF16),
            pltpu.VMEM((2, M, D), F32),
            pltpu.VMEM((2, M, D), BF16),
            pltpu.SemaphoreType.DMA((2 * NC,)),
            pltpu.SemaphoreType.DMA((NT,)),
            pltpu.SemaphoreType.DMA((NT,)),
            pltpu.SemaphoreType.DMA((NT,)),
            pltpu.SemaphoreType.DMA((NT,)),
            pltpu.SemaphoreType.DMA((5 * HPB,)),
            pltpu.SemaphoreType.DMA((NC + TAILSPLIT,)),
        ],
        compiler_params=pltpu.CompilerParams(vmem_limit_bytes=110 * 1024 * 1024, disable_bounds_checks=True,
                                             disable_semaphore_checks=True),
    )(A_x.reshape(M, D), A_k, A_v, A_wq, A_wo, B_x.reshape(M, D), B_k, B_v, B_wq, B_wo)
    return out.reshape(B, SQ, 2 * D)


@jax.jit
def pallas_concat_heads__mha_block_cached__mha_block_cached__near_ridge_kernel(
        A_x, A_k_cache, A_v_cache, A_wq, A_wo, B_x, B_k_cache, B_v_cache, B_wq, B_wo):
    return impl(A_x, A_k_cache, A_v_cache, A_wq, A_wo, B_x, B_k_cache, B_v_cache, B_wq, B_wo)
```

```python
import jax
import jax.numpy as jnp
import jax.experimental.pallas as pl
import jax.experimental.pallas.tpu as pltpu

B, SQ, D = 16, 80, 512
H, SK, DH = 32, 80, 128
M = B * SQ
HPB = 4
TPB = H // HPB
NT = 2 * TPB
NC = 4
BPC = B // NC
RC = BPC * SQ
UPB = HPB * NC
OR = 4
TAIL = 4
EXP2_SCALE = (DH ** -0.5) * 1.4426950408889634
F32 = jnp.float32
BF16 = jnp.bfloat16


def _kernel(ax, ak, av, awq, awo, bx, bk, bv, bwq, bwo, out_hbm,
            x_all, k_all, v_all, wq_all, wo_all, q_buf, o_ring, p_buf, acc, stage,
            sem_x, sem_k, sem_v, sem_wq, sem_wo, sem_h, sem_out):

    def times(i, n):
        return i * n if isinstance(i, int) else pl.multiple_of(i * n, n)

    def grp_copy(name, t, br):
        kk, vv, wq, wo = (ak, av, awq, awo) if br == 0 else (bk, bv, bwq, bwo)
        h0 = (t - br * TPB) * HPB
        if name == "k":
            return pltpu.make_async_copy(kk.at[:, pl.ds(h0, HPB)], k_all.at[t], sem_k.at[t])
        if name == "v":
            return pltpu.make_async_copy(vv.at[:, pl.ds(h0, HPB)], v_all.at[t], sem_v.at[t])
        if name == "wq":
            return pltpu.make_async_copy(wq.at[:, pl.ds(times(h0, DH), HPB * DH)], wq_all.at[t], sem_wq.at[t])
        return pltpu.make_async_copy(wo.at[pl.ds(times(h0, DH), HPB * DH), :], wo_all.at[t], sem_wo.at[t])

    def start_grp(names, t):
        if isinstance(t, int):
            for n in names:
                grp_copy(n, t, t // TPB).start()
            return

        @pl.when(t < TPB)
        def _():
            for n in names:
                grp_copy(n, t, 0).start()

        @pl.when(jnp.logical_and(t >= TPB, t < NT))
        def _():
            for n in names:
                grp_copy(n, t, 1).start()

    def wait_grp(buf, sem, t):
        pltpu.make_async_copy(buf.at[t], buf.at[t], sem.at[t]).wait()

    def head_copy(name, j):
        cols = pl.ds(times(j, DH), DH)
        if name == "wq0":
            return pltpu.make_async_copy(awq.at[:, cols], wq_all.at[0, :, cols], sem_h.at[j])
        if name == "wq1":
            return pltpu.make_async_copy(awq.at[:, pl.ds(times(HPB + j, DH), DH)], wq_all.at[1, :, cols],
                                         sem_h.at[HPB + j])
        if name == "k":
            return pltpu.make_async_copy(ak.at[:, j], k_all.at[0, :, j], sem_h.at[2 * HPB + j])
        if name == "v":
            return pltpu.make_async_copy(av.at[:, j], v_all.at[0, :, j], sem_h.at[3 * HPB + j])
        return pltpu.make_async_copy(awo.at[cols, :], wo_all.at[0, cols, :], sem_h.at[4 * HPB + j])

    def xa_copy(c):
        rows = pl.ds(times(c, RC), RC)
        return pltpu.make_async_copy(ax.at[rows], x_all.at[0, rows], sem_x.at[c])

    def xb_copy():
        return pltpu.make_async_copy(bx, x_all.at[1], sem_x.at[NC])

    def out_copy(br, r0, nr, s):
        return pltpu.make_async_copy(stage.at[br, pl.ds(r0, nr)],
                                     out_hbm.at[pl.ds(r0, nr), pl.ds(br * D, D)], sem_out.at[s])

    def q_proj(u, t):
        j, c = divmod(u, NC)
        q = jnp.dot(x_all[t // TPB, pl.ds(c * RC, RC), :], wq_all[t, :, pl.ds(j * DH, DH)],
                    preferred_element_type=F32)
        q_buf[u] = q.astype(BF16)

    def scores_softmax(u, t):
        j, c = divmod(u, NC)
        res = []
        for i in range(BPC):
            s = jax.lax.dot_general(q_buf[u, pl.ds(i * SQ, SQ), :], k_all[t, c * BPC + i, j],
                                    (((1,), (1,)), ((), ())), preferred_element_type=F32)
            m = jnp.max(s, axis=-1, keepdims=True)
            p = jnp.exp2((s - m) * EXP2_SCALE)
            l = jnp.sum(p, axis=-1, keepdims=True)
            r = pl.reciprocal(l, approx=True)
            r = r * (2.0 - l * r)
            res.append((p, r))
        return res

    def p_times_v(pr, u, t, slot):
        j, c = divmod(u, NC)
        for i in range(BPC):
            p, r = pr[i]
            o = jnp.dot(p.astype(BF16), v_all[t, c * BPC + i, j], preferred_element_type=F32)
            o_ring[slot, pl.ds(i * SQ, SQ), :] = (o * r).astype(BF16)

    def out_proj(u, t, slot, mode="acc", r0=0, nr=RC):
        j, c = divmod(u, NC)
        br = t // TPB
        part = jnp.dot(o_ring[slot, pl.ds(r0, nr), :], wo_all[t, pl.ds(j * DH, DH), :],
                       preferred_element_type=F32)
        rows = pl.ds(c * RC + r0, nr)
        if mode == "init":
            acc[br, rows, :] = part
        elif mode == "final":
            stage[br, rows, :] = (acc[br, rows, :] + part).astype(BF16)
        else:
            new = acc[br, rows, :] + part
            acc[br, rows, :] = new
            if j == HPB - 1:
                stage[br, rows, :] = new.astype(BF16)

    LAST = UPB - 1

    def stash_last(pr):
        for i in range(BPC):
            p, r = pr[i]
            p_buf[i] = (p * r).astype(BF16)

    def finish_previous(t):
        j, c = divmod(LAST, NC)
        for i in range(BPC):
            o = jnp.dot(p_buf[i], v_all[t - 1, c * BPC + i, j], preferred_element_type=F32)
            o_ring[LAST % OR, pl.ds(i * SQ, SQ), :] = o.astype(BF16)
        out_proj(LAST - 1, t - 1, (LAST - 1) % OR)

    def group(t, first):
        if not first:
            finish_previous(t)
        for u in range(UPB):
            j, c = divmod(u, NC)
            if first and c == 0 and j % 2 == 0:
                for jj in (j, j + 1):
                    for n in ("k", "v", "wq1", "wo"):
                        head_copy(n, jj).wait()
            if u == 1:
                start_grp(["k", "v", "wo"], t + 2)
                start_grp(["wq"], t + 3)
                if first:
                    xb_copy().start()
                else:
                    @pl.when(t == TPB)
                    def _():
                        out_copy(0, 0, M, 0).start()
            pr = scores_softmax(u, t)
            q_proj(u, t + 1)
            if u == LAST:
                stash_last(pr)
                continue
            p_times_v(pr, u, t, u % OR)
            if u >= 1:
                out_proj(u - 1, t, (u - 1) % OR, "init" if first and u - 1 < NC else "acc")
            elif not first:
                out_proj(LAST, t - 1, LAST % OR)

    xa_copy(0).start()
    head_copy("wq0", 0).start()

    def _start_wq0(j, carry):
        head_copy("wq0", j).start()
        return carry
    jax.lax.fori_loop(1, HPB, _start_wq0, 0)

    def _start_x(c, carry):
        xa_copy(c).start()
        return carry
    jax.lax.fori_loop(1, NC, _start_x, 0)

    def _start_head(j, carry):
        for n in ("k", "v", "wq1", "wo"):
            head_copy(n, j).start()
        return carry
    jax.lax.fori_loop(0, HPB, _start_head, 0)
    start_grp(["k", "v", "wo"], 1)
    start_grp(["wq"], 2)

    acc[1] = jnp.zeros(acc.shape[1:], F32)

    half = HPB // 2
    xa_copy(0).wait()
    for j in range(half):
        head_copy("wq0", j).wait()
    for j in range(half):
        q_proj(j * NC, 0)
    for j in range(half, HPB):
        head_copy("wq0", j).wait()
    xa_copy(1).wait()
    for j in range(half, HPB):
        q_proj(j * NC, 0)
    for j in range(HPB):
        q_proj(j * NC + 1, 0)
    xa_copy(2).wait()
    xa_copy(3).wait()
    for c in range(2, NC):
        for j in range(HPB):
            q_proj(j * NC + c, 0)

    group(0, first=True)

    def body(t, carry):
        wait_grp(k_all, sem_k, t)
        wait_grp(v_all, sem_v, t)
        wait_grp(wo_all, sem_wo, t)
        wait_grp(wq_all, sem_wq, t + 1)

        @pl.when(t == TPB - 1)
        def _():
            xb_copy().wait()

        group(t, first=False)
        return carry

    jax.lax.fori_loop(1, NT - 1, body, 0)

    t = NT - 1
    wait_grp(k_all, sem_k, t)
    wait_grp(v_all, sem_v, t)
    wait_grp(wo_all, sem_wo, t)
    order = [j * NC + c for c in range(NC) for j in range(HPB)]
    piece = RC // TAIL

    def out_last(i):
        if i < 0:
            out_proj(LAST, t - 1, LAST % OR)
            return
        u = order[i]
        j, c = divmod(u, NC)
        if j < HPB - 1:
            out_proj(u, t, i % OR)
        elif c < NC - 1:
            out_proj(u, t, i % OR, "final")
            out_copy(1, c * RC, RC, 1 + c).start()
        else:
            for s in range(TAIL):
                out_proj(u, t, i % OR, "final", r0=s * piece, nr=piece)
                out_copy(1, c * RC + s * piece, piece, NC + s).start()

    finish_previous(t)
    pending = {0: scores_softmax(order[0], t), 1: scores_softmax(order[1], t)}
    out_last(-1)
    p_times_v(pending.pop(0), order[0], t, 0)
    for i in range(2, UPB):
        pending[i] = scores_softmax(order[i], t)
        p_times_v(pending.pop(i - 1), order[i - 1], t, (i - 1) % OR)
        out_last(i - 2)
    p_times_v(pending.pop(UPB - 1), order[UPB - 1], t, (UPB - 1) % OR)
    out_last(UPB - 2)
    out_last(UPB - 1)

    out_copy(0, 0, M, 0).wait()
    for c in range(NC - 1):
        out_copy(1, c * RC, RC, 1 + c).wait()
    for s in range(TAIL):
        out_copy(1, (NC - 1) * RC + s * piece, piece, NC + s).wait()


@jax.jit
def pallas_concat_heads__mha_block_cached__mha_block_cached__near_ridge_kernel(
        A_x, A_k_cache, A_v_cache, A_wq, A_wo, B_x, B_k_cache, B_v_cache, B_wq, B_wo):
    hbm = pl.BlockSpec(memory_space=pl.ANY)
    out = pl.pallas_call(
        _kernel,
        in_specs=[hbm] * 10,
        out_specs=hbm,
        out_shape=jax.ShapeDtypeStruct((M, 2 * D), BF16),
        scratch_shapes=[
            pltpu.VMEM((2, M, D), BF16),
            pltpu.VMEM((NT, B, HPB, SK, DH), BF16),
            pltpu.VMEM((NT, B, HPB, SK, DH), BF16),
            pltpu.VMEM((NT, D, HPB * DH), BF16),
            pltpu.VMEM((NT, HPB * DH, D), BF16),
            pltpu.VMEM((UPB, RC, DH), BF16),
            pltpu.VMEM((OR, RC, DH), BF16),
            pltpu.VMEM((BPC, SQ, SK), BF16),
            pltpu.VMEM((2, M, D), F32),
            pltpu.VMEM((2, M, D), BF16),
            pltpu.SemaphoreType.DMA((NC + 1,)),
            pltpu.SemaphoreType.DMA((NT,)),
            pltpu.SemaphoreType.DMA((NT,)),
            pltpu.SemaphoreType.DMA((NT,)),
            pltpu.SemaphoreType.DMA((NT,)),
            pltpu.SemaphoreType.DMA((5 * HPB,)),
            pltpu.SemaphoreType.DMA((NC + TAIL,)),
        ],
        compiler_params=pltpu.CompilerParams(
            vmem_limit_bytes=110 * 1024 * 1024,
            disable_bounds_checks=True,
            disable_semaphore_checks=True,
        ),
    )(A_x.reshape(M, D), A_k_cache, A_v_cache, A_wq, A_wo,
      B_x.reshape(M, D), B_k_cache, B_v_cache, B_wq, B_wo)
    return out.reshape(B, SQ, 2 * D)
```
